```python
import os as _os
_os.environ.setdefault("JAX_PLATFORMS", "cpu")
import jax
import jax.numpy as jnp

def _softmax(x, axis=-1):
    return jax.nn.softmax(x, axis=axis)
def _gelu(x):
    return jax.nn.gelu(x, approximate=True)
def _silu(x):
    return jax.nn.silu(x)
def _sigmoid(x):
    return jax.nn.sigmoid(x)
def _layernorm(x, axis=-1, eps=1e-5):
    m = jnp.mean(x, axis=axis, keepdims=True)
    v = jnp.var(x, axis=axis, keepdims=True)
    return (x - m) / jnp.sqrt(v + eps)
def _scatter_add(tgt, idx, src, axis=0):
    return tgt.at[idx].add(src)
def _segment_sum(src, seg, n):
    return jax.ops.segment_sum(src, seg, n)
class _Rng:
    def __init__(self, key):
        self._k = key
    def _next(self):
        self._k, sub = jax.random.split(self._k)
        return sub
    def normal(self, shape):
        return jax.random.normal(self._next(), shape, dtype=jnp.bfloat16)
    def randint(self, lo, hi, shape):
        return jax.random.randint(self._next(), shape, lo, hi, dtype=jnp.int32)
    def uniform(self, shape, lo=0.0, hi=1.0):
        return jax.random.uniform(self._next(), shape, jnp.bfloat16, lo, hi)
    def permutation(self, n):
        return jax.random.permutation(self._next(), n)


kernel_name = 'standalone__mha_softmax__near_ridge'

def setup_inputs():
    _rng = _Rng(jax.random.key(int.from_bytes(__import__("os").urandom(4), "little")))
    _w = (lambda a: (lambda t: t.astype(jnp.bfloat16) if jnp.issubdtype(t.dtype, jnp.floating) else t)(jnp.asarray(a)))
    B, H, Sq, Sk, D = 8, 16, 192, 1024, 256
    return {
        "q": _w((lambda *s: _rng.normal(s) * 0.4)(B, H, Sq, D)),
        "k": _w((lambda *s: _rng.normal(s) * 0.4)(B, H, Sk, D)),
        "v": _w((lambda *s: _rng.normal(s) * 0.05)(B, H, Sk, D)),
    }

def reference(q, k, v):
    scale = q.shape[-1] ** -0.5
    scores = jnp.einsum("bhqd,bhkd->bhqk", q, k) * scale
    p = _softmax(scores, axis=-1)
    return jnp.einsum("bhqk,bhkd->bhqd", p, v)
```

```python
import jax
import jax.numpy as jnp
from jax import lax
import jax.experimental.pallas as pl
import jax.experimental.pallas.tpu as pltpu

_RING = 3
_NT = (((1,), (1,)), ((), ()))


def _attend(q, k, v, scale):
    s = lax.dot_general(q, k, _NT, preferred_element_type=jnp.float32)
    m = jnp.max(s, axis=-1, keepdims=True)
    p = jnp.exp((s - m) * scale)
    l = jnp.sum(p, axis=-1, keepdims=True)
    o = jnp.dot(p.astype(v.dtype), v, preferred_element_type=jnp.float32)
    return o / l


@jax.jit
def pallas_standalone__mha_softmax__near_ridge_kernel(
    q: jax.Array,
    k: jax.Array,
    v: jax.Array,
):
    B, H, Sq, D = q.shape
    Sk = k.shape[2]
    N = B * H
    scale = D ** -0.5
    ring = min(_RING, N)

    def kernel_function(q_hbm, k_hbm, v_hbm, o_hbm, q_buf, k_buf, v_buf, o_buf,
                        in_sems, out_sems):
        def loads(h, slot):
            return (
                (pltpu.make_async_copy(q_hbm.at[h], q_buf.at[slot], in_sems.at[0, slot]), 0),
                (pltpu.make_async_copy(k_hbm.at[h], k_buf.at[slot], in_sems.at[1, slot]), 0),
                (pltpu.make_async_copy(v_hbm.at[h], v_buf.at[slot], in_sems.at[2, slot]), 1),
            )

        bulk_store = pltpu.make_async_copy(
            o_buf.at[pl.ds(0, N - 1)], o_hbm.at[pl.ds(0, N - 1)], out_sems.at[0])
        last_store = pltpu.make_async_copy(
            o_buf.at[pl.ds(N - 1, 1)], o_hbm.at[pl.ds(N - 1, 1)], out_sems.at[1])

        for h in range(ring):
            for copy, priority in loads(h, h):
                copy.start(priority=priority)

        def body(h, carry):
            slot = h % ring
            for copy, _ in loads(h, slot):
                copy.wait()

            @pl.when(h == N - 1)
            def _():
                bulk_store.start()

            o_buf[h] = _attend(q_buf[slot], k_buf[slot], v_buf[slot], scale).astype(o_buf.dtype)

            @pl.when(h + ring < N)
            def _():
                for copy, priority in loads(h + ring, slot):
                    copy.start(priority=priority)

            return carry

        lax.fori_loop(0, N, body, None)
        last_store.start(priority=1)
        bulk_store.wait()
        last_store.wait()

    out = pl.pallas_call(
        kernel_function,
        in_specs=[pl.BlockSpec(memory_space=pl.ANY)] * 3,
        out_specs=pl.BlockSpec(memory_space=pl.ANY),
        out_shape=jax.ShapeDtypeStruct((N, Sq, D), q.dtype),
        scratch_shapes=[
            pltpu.VMEM((ring, Sq, D), q.dtype),
            pltpu.VMEM((ring, Sk, D), k.dtype),
            pltpu.VMEM((ring, Sk, D), v.dtype),
            pltpu.VMEM((N, Sq, D), q.dtype),
            pltpu.SemaphoreType.DMA((3, ring)),
            pltpu.SemaphoreType.DMA((2,)),
        ],
        compiler_params=pltpu.CompilerParams(vmem_limit_bytes=64 * 1024 * 1024),
    )(q.reshape(N, Sq, D), k.reshape(N, Sk, D), v.reshape(N, Sk, D))
    return out.reshape(B, H, Sq, D)
```

```python
import math

import jax
import jax.numpy as jnp
from jax import lax
import jax.experimental.pallas as pl
import jax.experimental.pallas.tpu as pltpu

_LANES = 8
_CHUNK_ROWS = 32
_SLOTS = 3
_NT = (((1,), (1,)), ((), ()))


def _start_alternating(copies):
    for i, copy in enumerate(copies):
        copy.start(priority=i % 2)


@jax.jit
def pallas_standalone__mha_softmax__near_ridge_kernel(
    q: jax.Array,
    k: jax.Array,
    v: jax.Array,
):
    B, H, Sq, D = q.shape
    Sk = k.shape[2]
    heads = B * H
    groups = heads // _LANES
    exp2_scale = D ** -0.5 * math.log2(math.e)

    q_rows, kv_rows = Sq // _LANES, Sk // _LANES
    ahead = _LANES + 2
    o_rows = (groups - 1) * Sq // ahead // _CHUNK_ROWS * _CHUNK_ROWS
    assert heads % _LANES == 0 and groups >= _SLOTS
    assert Sq % _CHUNK_ROWS == 0 and Sq % (8 * _LANES) == 0
    assert Sk % (_CHUNK_ROWS * _LANES) == 0
    assert 0 < (ahead - _LANES) * o_rows <= (groups - 2) * Sq

    def kernel_function(q_hbm, k_hbm, v_hbm, o_hbm, q_buf, k_buf, v_buf, o_buf,
                        load_sems, store_sem):
        hbms, bufs = (q_hbm, k_hbm, v_hbm), (q_buf, k_buf, v_buf)

        def start_loads(index):
            group, part = index // _LANES, index % _LANES
            slot = group % _SLOTS

            def load(which, lane, row, size):
                rows = pl.ds(pl.multiple_of(row, 8), size)
                return pltpu.make_async_copy(
                    hbms[which].at[lane, group, rows],
                    bufs[which].at[slot, lane, rows],
                    load_sems.at[which, slot, lane])

            copies = [load(0, lane, part * q_rows, q_rows) for lane in range(_LANES)]
            for row in range(0, kv_rows, _CHUNK_ROWS):
                for lane in range(_LANES):
                    for which in (1, 2):
                        copies.append(load(which, lane, part * kv_rows + row, _CHUNK_ROWS))
            _start_alternating(copies)

        def start_stores(first_row, size):
            _start_alternating(
                pltpu.make_async_copy(
                    o_buf.at[lane, pl.ds(first_row + row, _CHUNK_ROWS)],
                    o_hbm.at[lane, pl.ds(first_row + row, _CHUNK_ROWS)],
                    store_sem)
                for row in range(0, size, _CHUNK_ROWS)
                for lane in range(_LANES))

        def attend(step, start_copies):
            group, lane = step // _LANES, step % _LANES
            slot = group % _SLOTS
            for which, buf in enumerate(bufs):
                head = buf.at[slot, lane]
                pltpu.make_async_copy(head, head, load_sems.at[which, slot, lane]).wait()
            s = lax.dot_general(q_buf[slot, lane], k_buf[slot, lane], _NT,
                                preferred_element_type=jnp.float32)
            start_copies()
            p = jnp.exp2((s - jnp.max(s, axis=-1, keepdims=True)) * exp2_scale)
            denom = jnp.sum(p, axis=-1, keepdims=True)
            o = jnp.dot(p.astype(v_buf.dtype), v_buf[slot, lane],
                        preferred_element_type=jnp.float32)
            rows = pl.ds(pl.multiple_of(group * Sq, Sq), Sq)
            o_buf[lane, rows] = (o / denom).astype(o_buf.dtype)

        @pl.loop(0, ahead)
        def _(index):
            start_loads(index)

        @pl.loop(0, heads - ahead)
        def _(step):
            attend(step, lambda: start_loads(step + ahead))

        @pl.loop(0, ahead)
        def _(t):
            first_row = pl.multiple_of(t * o_rows, _CHUNK_ROWS)
            attend(heads - ahead + t, lambda: start_stores(first_row, o_rows))

        start_stores(ahead * o_rows, groups * Sq - ahead * o_rows)
        pltpu.make_async_copy(o_buf, o_hbm, store_sem).wait()

    out = pl.pallas_call(
        kernel_function,
        in_specs=[pl.BlockSpec(memory_space=pl.ANY)] * 3,
        out_specs=pl.BlockSpec(memory_space=pl.ANY),
        out_shape=jax.ShapeDtypeStruct((_LANES, groups * Sq, D), q.dtype),
        scratch_shapes=[
            pltpu.VMEM((_SLOTS, _LANES, Sq, D), q.dtype),
            pltpu.VMEM((_SLOTS, _LANES, Sk, D), k.dtype),
            pltpu.VMEM((_SLOTS, _LANES, Sk, D), v.dtype),
            pltpu.VMEM((_LANES, groups * Sq, D), q.dtype),
            pltpu.SemaphoreType.DMA((3, _SLOTS, _LANES)),
            pltpu.SemaphoreType.DMA(()),
        ],
        compiler_params=pltpu.CompilerParams(
            vmem_limit_bytes=64 * 1024 * 1024,
            disable_bounds_checks=True,
            disable_semaphore_checks=True,
        ),
    )(
        q.reshape(_LANES, groups, Sq, D),
        k.reshape(_LANES, groups, Sk, D),
        v.reshape(_LANES, groups, Sk, D),
    )
    return out.reshape(B, H, Sq, D)
```
